```python
import os as _os
_os.environ.setdefault("JAX_PLATFORMS", "cpu")
import jax
import jax.numpy as jnp

def _softmax(x, axis=-1):
    return jax.nn.softmax(x, axis=axis)
def _gelu(x):
    return jax.nn.gelu(x, approximate=True)
def _silu(x):
    return jax.nn.silu(x)
def _sigmoid(x):
    return jax.nn.sigmoid(x)
def _layernorm(x, axis=-1, eps=1e-5):
    m = jnp.mean(x, axis=axis, keepdims=True)
    v = jnp.var(x, axis=axis, keepdims=True)
    return (x - m) / jnp.sqrt(v + eps)
def _scatter_add(tgt, idx, src, axis=0):
    return tgt.at[idx].add(src)
def _segment_sum(src, seg, n):
    return jax.ops.segment_sum(src, seg, n)
class _Rng:
    def __init__(self, key):
        self._k = key
    def _next(self):
        self._k, sub = jax.random.split(self._k)
        return sub
    def normal(self, shape):
        return jax.random.normal(self._next(), shape, dtype=jnp.bfloat16)
    def randint(self, lo, hi, shape):
        return jax.random.randint(self._next(), shape, lo, hi, dtype=jnp.int32)
    def uniform(self, shape, lo=0.0, hi=1.0):
        return jax.random.uniform(self._next(), shape, jnp.bfloat16, lo, hi)
    def permutation(self, n):
        return jax.random.permutation(self._next(), n)


kernel_name = 'parallel_sum__mha_block__swiglu_ffn__prompt'

def setup_inputs():
    _rng = _Rng(jax.random.key(int.from_bytes(__import__("os").urandom(4), "little")))
    _w = (lambda a: (lambda t: t.astype(jnp.bfloat16) if jnp.issubdtype(t.dtype, jnp.floating) else t)(jnp.asarray(a)))
    def _A_setup():
        B, S, D, H = 1, 2048, 640, 32
        return {
            "x": _w((lambda *s: _rng.normal(s) * 0.05)(B, S, D)),
            "wqkv": _w((lambda *s: _rng.normal(s) * 0.1)(D, 3 * D)),
            "wo": _w((lambda *s: _rng.normal(s) * 0.05)(D, D)),
        }
    _A_in = _A_setup()

    def _B_setup():
        B, S, D, F = 1, 2048, 640, 1536
        return {
            "x": _w((lambda *s: _rng.normal(s) * 0.05)(B, S, D)),
            "w_gate": _w((lambda *s: _rng.normal(s) * 0.05)(D, F)),
            "w_up": _w((lambda *s: _rng.normal(s) * 0.05)(D, F)),
            "w_down": _w((lambda *s: _rng.normal(s) * 0.05)(F, D)),
        }
    _B_in = _B_setup()

    return {
        "A_x": _A_in["x"],
        "A_wqkv": _A_in["wqkv"],
        "A_wo": _A_in["wo"],
        "B_x": _B_in["x"],
        "B_w_gate": _B_in["w_gate"],
        "B_w_up": _B_in["w_up"],
        "B_w_down": _B_in["w_down"],
    }

def reference(A_x, A_wqkv, A_wo, B_x, B_w_gate, B_w_up, B_w_down):
    def _A_ref(x, wqkv, wo):
        B, S, D = x.shape
        H = 32
        Dh = D // H
        qkv = (lambda x, *d: x.transpose(*d))((x @ wqkv).reshape(B, S, 3, H, Dh), 2, 0, 3, 1, 4)
        q, k, v = qkv[0], qkv[1], qkv[2]
        scores = jnp.einsum("bhqd,bhkd->bhqk", q, k) * (Dh ** -0.5)
        p = _softmax(scores, axis=-1)
        o = jnp.einsum("bhqk,bhkd->bhqd", p, v)
        return (lambda x, *d: x.transpose(*d))(o, 0, 2, 1, 3).reshape(B, S, D) @ wo

    def _B_ref(x, w_gate, w_up, w_down):
        g = _silu(x @ w_gate)
        u = x @ w_up
        return (g * u) @ w_down

    x = A_x
    xn = _layernorm(x, axis=-1)
    return x + _A_ref(xn, A_wqkv, A_wo) + _B_ref(xn, B_w_gate, B_w_up, B_w_down)
```

```python
import math

import jax
import jax.numpy as jnp
from jax import lax
from jax.experimental import pallas as pl
from jax.experimental.pallas import tpu as pltpu

H = 32
EPS = 1e-5
LANES = 128
RB = 512
BQ = 1024
GQ = 512
CK = 128
VR = 24

F32 = jnp.float32
BF16 = jnp.bfloat16


def _dot(a, b, dims=((1,), (0,))):
    return lax.dot_general(a, b, (dims, ((), ())), preferred_element_type=F32)


def _kernel(
    x_hbm, wqkv_hbm, wo_hbm, wg_hbm, wu_hbm, wd_hbm,
    out_hbm,
    x_v, wqkv_v, wo_v, wg_v, wu_v, wd_v,
    xn_v, kw_v, qt_v, vt_v, ot_v, sa_v, sb_v, m_v, out_v,
    x_sem, w_sem, out_sem,
):
    S, D = x_v.shape
    DH = D // H
    NT = D // LANES
    NRB = S // RB
    NG = BQ // GQ
    NC = S // CK
    NQB = S // BQ
    q_scale = DH ** -0.5 * math.log2(math.e)

    def x_copy(r):
        rows = pl.ds(r * RB, RB)
        return pltpu.make_async_copy(x_hbm.at[rows], x_v.at[rows], x_sem.at[r])

    w_copies = [
        pltpu.make_async_copy(src, dst, w_sem.at[i])
        for i, (src, dst) in enumerate(
            [(wqkv_hbm, wqkv_v), (wo_hbm, wo_v), (wg_hbm, wg_v),
             (wu_hbm, wu_v), (wd_hbm, wd_v)])
    ]
    x_copy(0).start()
    w_copies[0].start()
    for r in range(1, NRB):
        x_copy(r).start()

    def project(r):
        rows = pl.ds(pl.multiple_of(r * RB, RB), RB)
        x = x_v[rows, :].astype(F32)
        xc = x - jnp.mean(x, axis=-1, keepdims=True)
        var = jnp.mean(xc * xc, axis=-1, keepdims=True)
        xn = (xc / jnp.sqrt(var + EPS)).astype(BF16)
        xn_v[rows, :] = xn
        k = _dot(xn, wqkv_v[:, D:2 * D]).astype(BF16)
        upper = lax.broadcasted_iota(jnp.int32, (RB, LANES), 1) >= LANES // 2
        for j in range(NT):
            kj = k[:, j * LANES:(j + 1) * LANES]
            kw_v[2 * j, rows, :] = kj
            if j + 1 < NT:
                kw_v[2 * j + 1, rows, :] = jnp.where(
                    upper, kj, k[:, (j + 1) * LANES:(j + 2) * LANES])
        qt = _dot(wqkv_v[:, :D], xn, ((0,), (1,)))
        qt_v[r] = (qt * q_scale).astype(BF16)
        vt = _dot(wqkv_v[:, 2 * D:], xn, ((0,), (1,)))
        vt_v[r] = vt.astype(BF16).astype(F32)

    x_copy(0).wait()
    w_copies[0].wait()
    for c in w_copies[1:]:
        c.start()
    project(0)

    def project_body(r, carry):
        x_copy(r).wait()
        project(r)
        return carry

    lax.fori_loop(1, NRB, project_body, 0)

    def head_q(h, col):
        lo = h * DH
        top = ((lo + DH - 1) // LANES) * LANES
        bot = (lo // LANES) * LANES + LANES // 2
        q = jnp.concatenate(
            [qt_v[col, pl.ds(pl.multiple_of(top, LANES // 2), LANES // 2), :],
             qt_v[col, pl.ds(pl.multiple_of(bot, LANES // 2), LANES // 2), :]],
            axis=0)
        row = lax.broadcasted_iota(jnp.int32, q.shape, 0)
        return jnp.where(((row - lo) & (LANES - 1)) < DH, q, jnp.zeros_like(q))

    def scores(h, q, g, c, s_ref, m):
        w = (h * DH) // LANES + (h * DH + DH - 1) // LANES
        keys = pl.ds(c * CK, CK)
        s = _dot(kw_v[w, keys, :], q)
        s_ref[g, keys, :] = s
        mc = jnp.max(s.reshape(CK // 8, 8, GQ), axis=0)
        return mc if m is None else jnp.maximum(m, mc)

    def values(h, odd, g, c, s_ref, m, acc):
        p = jnp.exp2(s_ref[g, pl.ds(c * CK, CK), :] - m).astype(BF16)
        base = pl.multiple_of((h * DH) // 8 * 8, 8)
        r, lo = divmod(c * CK, RB)
        vt = vt_v[r, pl.ds(base, VR), pl.ds(lo, CK)]
        row = lax.broadcasted_iota(jnp.int32, vt.shape, 0)
        spare = (row < VR - DH) if odd else (row >= DH)
        o = _dot(jnp.where(spare, 1.0, vt), p)
        return o if acc is None else acc + o

    def finish(h, odd, col, acc):
        base = pl.multiple_of((h * DH) // 8 * 8, 8)
        lrow = 0 if odd else VR - 1
        o = acc * (1.0 / acc[lrow:lrow + 1, :])
        if odd:
            row = lax.broadcasted_iota(jnp.int32, (8, GQ), 0)
            first = jnp.where(
                row < VR - DH, ot_v[col, pl.ds(base, 8), :], o[:8])
            o = jnp.concatenate([first, o[8:]], axis=0)
        ot_v[col, pl.ds(base, VR), :] = o

    def step(nxt, cur, odd, s_nxt, s_cur):
        for g in range(NG):
            m = acc = None
            if nxt is not None:
                hn = nxt % H
                q = head_q(hn, (nxt // H) * NG + g)
            if cur is not None:
                hc = cur % H
                m_cur = m_v[g] if False else m_v[g, 0:1, :]
            for c in range(NC):
                if nxt is not None:
                    m = scores(hn, q, g, c, s_nxt, m)
                if cur is not None:
                    acc = values(hc, odd, g, c, s_cur, m_cur, acc)
            if cur is not None:
                finish(hc, odd, (cur // H) * NG + g, acc)
            if nxt is not None:
                m_v[g] = jnp.broadcast_to(
                    jnp.max(m, axis=0, keepdims=True), (8, GQ))

    n_items = NQB * H
    step(0, None, False, sa_v, None)

    def attn_body(i, carry):
        @pl.when(i % 2 == 0)
        def _():
            step(i + 1, i, False, sb_v, sa_v)

        @pl.when(i % 2 == 1)
        def _():
            step(i + 1, i, True, sa_v, sb_v)

        return carry

    lax.fori_loop(0, n_items - 1, attn_body, 0)
    step(None, n_items - 1, True, None, sb_v)

    for c in w_copies[1:]:
        c.wait()

    def out_copy(r):
        rows = pl.ds(pl.multiple_of(r * RB, RB), RB)
        return pltpu.make_async_copy(
            out_v.at[rows], out_hbm.at[rows], out_sem.at[r])

    def out_body(r, carry):
        rows = pl.ds(pl.multiple_of(r * RB, RB), RB)
        xn = xn_v[rows, :]
        g = _dot(xn, wg_v[...])
        u = _dot(xn, wu_v[...])
        hid = (g * jax.nn.sigmoid(g) * u).astype(BF16)
        y = _dot(ot_v[r].astype(BF16), wo_v[...], ((0,), (0,)))
        y = y + _dot(hid, wd_v[...])
        out_v[rows, :] = (x_v[rows, :].astype(F32) + y).astype(out_v.dtype)
        out_copy(r).start()
        return carry

    lax.fori_loop(0, NRB, out_body, 0)
    for r in range(NRB):
        out_copy(r).wait()


@jax.jit
def pallas_parallel_sum__mha_block__swiglu_ffn__prompt_kernel(
    A_x: jax.Array,
    A_wqkv: jax.Array,
    A_wo: jax.Array,
    B_x: jax.Array,
    B_w_gate: jax.Array,
    B_w_up: jax.Array,
    B_w_down: jax.Array,
):
    del B_x
    B, S, D = A_x.shape
    assert B == 1 and D == 20 * H and S % BQ == 0 and RB == GQ
    weights = (A_wqkv, A_wo, B_w_gate, B_w_up, B_w_down)
    nrb = S // RB
    any_spec = pl.BlockSpec(memory_space=pl.ANY)
    out = pl.pallas_call(
        _kernel,
        out_shape=jax.ShapeDtypeStruct((S, D), A_x.dtype),
        in_specs=[any_spec] * 6,
        out_specs=any_spec,
        scratch_shapes=[
            pltpu.VMEM((S, D), A_x.dtype),
            *[pltpu.VMEM(w.shape, w.dtype) for w in weights],
            pltpu.VMEM((S, D), BF16),
            pltpu.VMEM((2 * (D // LANES) - 1, S, LANES), BF16),
            pltpu.VMEM((nrb, D, RB), BF16),
            pltpu.VMEM((nrb, D, RB), F32),
            pltpu.VMEM((nrb, D, RB), F32),
            pltpu.VMEM((BQ // GQ, S, GQ), F32),
            pltpu.VMEM((BQ // GQ, S, GQ), F32),
            pltpu.VMEM((BQ // GQ, 8, GQ), F32),
            pltpu.VMEM((S, D), A_x.dtype),
            pltpu.SemaphoreType.DMA((nrb,)),
            pltpu.SemaphoreType.DMA((len(weights),)),
            pltpu.SemaphoreType.DMA((nrb,)),
        ],
        compiler_params=pltpu.CompilerParams(
            vmem_limit_bytes=110 * 1024 * 1024),
        name="mha_swiglu_parallel",
    )(A_x.reshape(S, D), *weights)
    return out.reshape(B, S, D)
```

```python
import contextlib
import math

import jax
import jax.numpy as jnp
from jax import lax
from jax.experimental import pallas as pl
from jax.experimental.pallas import tpu as pltpu

scope = lambda n: contextlib.nullcontext()

H = 32
EPS = 1e-5
LANES = 128
RB = 512
CK = 128
UK = 16
NU = 11
NX = 3
NU0 = 0
LEAD = 20
XLEAD = 20
PF32 = 1
VR = 24
KH = 256

F32 = jnp.float32
BF16 = jnp.bfloat16
I32 = jnp.int32


def _dot(a, b, dims=((1,), (0,))):
    return lax.dot_general(a, b, (dims, ((), ())), preferred_element_type=F32)


def _lane_gather(x, idx):
    return lax.gather(
        x, idx[..., None],
        lax.GatherDimensionNumbers(
            offset_dims=(), collapsed_slice_dims=(1,), start_index_map=(1,),
            operand_batching_dims=(0,), start_indices_batching_dims=(0,)),
        slice_sizes=(1, 1), mode=lax.GatherScatterMode.PROMISE_IN_BOUNDS)


def _fold_max(m, s):
    s = jnp.max(s.reshape(-1, 8, s.shape[-1]), axis=0)
    return s if m is None else jnp.maximum(m, s)


class _Background:
    def __init__(self, never, n_ticks, lead):
        self.never, self.n_ticks, self.lead = never, n_ticks, lead
        self.jobs, self.ticks, self.done = [], [], 0

    def tick(self, result, share=1.0):
        n = result.shape[0] // 8
        keep = round(n * share)
        self.ticks += [result[8 * (i * n // keep):][:8, :LANES]
                       for i in range(keep)]

    def run(self, last=False):
        while self.done < len(self.jobs):
            t = self.done * self.n_ticks // len(self.jobs) - self.lead
            if t >= len(self.ticks) and not last:
                break

            def after(x):
                if t < 0:
                    return x
                reps = (x.shape[0] // 8, x.shape[1] // LANES)
                tick = pltpu.bitcast(self.ticks[min(t, len(self.ticks) - 1)], I32)
                return jnp.where(
                    jnp.tile(self.never, reps) != 0, jnp.tile(tick, reps), x)

            self.jobs[self.done](after)
            self.done += 1


def _score_jobs(k, q_ref, emit):
    dh, nq = q_ref.shape
    acc = []

    def job(d, after):
        idx = after(jnp.full((8, LANES), d, I32))
        kd = [_lane_gather(k[a:a + 8], idx) for a in range(0, UK, 8)]
        qd = [q_ref[d:d + 1, j:j + LANES] for j in range(0, nq, LANES)]
        jobs = [[ka * qj for qj in qd] for ka in kd]
        acc[:] = jobs if d == 0 else [
            [x + y for x, y in zip(xs, ys)] for xs, ys in zip(acc, jobs)]
        if d == dh - 1:
            emit(jnp.concatenate(
                [jnp.concatenate(xs, axis=1) for xs in acc], axis=0))

    return [lambda after, d=d: job(d, after) for d in range(dh)]


def _strassen_rhs_jobs(w_ref, sums_ref):
    _, k, n = sums_ref.shape

    def job(lo, col, after):
        b11, b12, b21, b22 = (
            pltpu.bitcast(after(pltpu.bitcast(
                w_ref[pl.ds(i * k + lo, 16), pl.ds(j * n + col, KH)], I32)),
                BF16).astype(F32)
            for i in range(2) for j in range(2))
        for i, b in enumerate(
                (b11 + b22, b12 - b22, b21 - b11, b11 + b12, b21 + b22)):
            sums_ref[i, pl.ds(lo, 16), pl.ds(col, KH)] = b.astype(BF16)

    return [lambda after, lo=lo, col=col: job(lo, col, after)
            for lo in range(0, k, 16) for col in range(0, n, KH)]


def _strassen_lhs(a11, a12, a21, a22):
    f11, f12, f21, f22 = (t.astype(F32) for t in (a11, a12, a21, a22))
    return [t.astype(BF16) for t in (
        f11 + f22, f21 + f22, a11, a22, f11 + f12, f21 - f11, f12 - f22)]


def _strassen(lhs, w_ref, sums_ref, i, j, dot):
    _, k, n = sums_ref.shape

    def block_sum(t):
        return sums_ref[t, pl.ds(i, KH), pl.ds(j, KH)]

    m1 = dot(lhs[0], block_sum(0))
    m2 = dot(lhs[1], w_ref[pl.ds(i, KH), pl.ds(j, KH)])
    m3 = dot(lhs[2], block_sum(1))
    m4 = dot(lhs[3], block_sum(2))
    m5 = dot(lhs[4], w_ref[pl.ds(k + i, KH), pl.ds(n + j, KH)])
    m6 = dot(lhs[5], block_sum(3))
    m7 = dot(lhs[6], block_sum(4))
    return [m1, m2, m3, m4, m5, m6, m7]


def _strassen_combine(m1, m2, m3, m4, m5, m6, m7):
    return jnp.concatenate(
        [jnp.concatenate([m1 + m4 - m5 + m7, m3 + m5], axis=1),
         jnp.concatenate([m2 + m4, m1 - m2 + m3 + m6], axis=1)], axis=0)


def _kernel(
    x_hbm, wqkv_hbm, wo_hbm, wg_hbm, wu_hbm, wd_hbm,
    out_hbm,
    x_v, wqkv_v, wo_v, wg_v, wu_v, wd_v,
    xn_v, wt_v, kw_v, qt_v, qh_v, qf_v, vt_v, ot_v, s_v, m_v, sx_v, mx_v, z_v,
    sg_v, su_v, sd_v, y_v, out_v,
    x_sem, qkv_sem, w_sem, out_sem,
):
    S, D = x_v.shape
    DH = D // H
    NT = D // LANES
    NB = S // RB
    NC = S // CK
    q_scale = DH ** -0.5 * math.log2(math.e)

    def x_copy(r):
        rows = pl.ds(r * RB, RB)
        return pltpu.make_async_copy(x_hbm.at[rows], x_v.at[rows], x_sem.at[r])

    def qkv_copy(i):
        cols = pl.ds(i * D, D)
        return pltpu.make_async_copy(
            wqkv_hbm.at[:, cols], wqkv_v.at[:, cols], qkv_sem.at[i])

    w_copies = [
        pltpu.make_async_copy(src, dst, w_sem.at[i])
        for i, (src, dst) in enumerate(
            [(wo_hbm, wo_v), (wg_hbm, wg_v), (wu_hbm, wu_v), (wd_hbm, wd_v)])
    ]

    def out_copy(r):
        rows = pl.ds(pl.multiple_of(r * RB, RB), RB)
        return pltpu.make_async_copy(
            out_v.at[rows], out_hbm.at[rows], out_sem.at[r])

    def loop(lo, hi, body):
        lax.fori_loop(lo, hi, lambda i, c: body(i), None)

    def layernorm(lo, n):
        rows = pl.ds(lo, n)
        x = x_v[rows, :].astype(F32)
        xc = x - jnp.mean(x, axis=-1, keepdims=True)
        var = jnp.mean(xc * xc, axis=-1, keepdims=True)
        xn = (xc * lax.rsqrt(var + EPS)).astype(BF16)
        xn_v[rows, :] = xn
        return xn

    def project_k(lo, xn):
        rows = pl.ds(lo, xn.shape[0])
        k = _dot(xn, wqkv_v[:, D:2 * D])
        lane = lax.broadcasted_iota(I32, (xn.shape[0], LANES), 1)
        for j in range(NT):
            kj = k[:, j * LANES:(j + 1) * LANES]
            kw_v[2 * j, rows, :] = kj.astype(BF16)
            if j + 1 < NT:
                kw_v[2 * j + 1, rows, :] = jnp.where(
                    lane >= LANES // 2, kj,
                    k[:, (j + 1) * LANES:(j + 2) * LANES]).astype(BF16)

    def project_qv(r):
        xn = xn_v[pl.ds(pl.multiple_of(r * RB, RB), RB), :]
        qv = _dot(wt_v[...], xn, ((1,), (1,)))
        qt = (qv[:D] * q_scale).astype(BF16)
        qt_v[r] = qt
        qt = qt.astype(F32)
        for h in range(H):
            qh_v[h, r] = qt[h * DH:(h + 1) * DH]
        vt_v[r] = qv[D:].astype(BF16).astype(F32)

    with scope("ph0"):
        x_copy(0).start()
        qkv_copy(1).start()
        z_v[...] = jnp.zeros_like(z_v)
        x_copy(0).wait()
        xn0 = layernorm(0, RB)
        for r in range(1, NB):
            x_copy(r).start()
        qkv_copy(1).wait()
        project_k(0, xn0)
        for r in range(1, NB):
            x_copy(r).wait()
        qkv_copy(0).start()
        qkv_copy(2).start()
        lo = RB
        for n in (128, 384, 512):
            project_k(lo, layernorm(lo, n))
            lo += n
        qkv_copy(0).wait()
        qkv_copy(2).wait()
        for c in w_copies:
            c.start()
        for n in (128, 384):
            project_k(lo, layernorm(lo, n))
            lo += n
        wt_v[:D, :] = wqkv_v[:, :D].T
        wt_v[D:, :] = wqkv_v[:, 2 * D:].T

    with scope("ph1_proj"):
        loop(0, NB, project_qv)

    def never():
        return pltpu.bitcast(z_v[:8, :LANES], I32)

    def window(h):
        return ((h * DH) >> 7) + ((h * DH + DH - 1) >> 7)

    def unit_keys(u):
        return pl.ds((u + 1) * CK - UK, UK)

    def to_lane0(k, h):
        return pltpu.roll(k.astype(F32), (-h * DH) & (LANES - 1), 1)

    def head_q(h, g):
        half = LANES // 2
        top = (h * DH + DH - 1) & -LANES
        bot = ((h * DH) & -LANES) + half
        q = jnp.concatenate(
            [qt_v[g, pl.ds(pl.multiple_of(top, half), half), :],
             qt_v[g, pl.ds(pl.multiple_of(bot, half), half), :]], axis=0)
        q = pltpu.bitcast(q, I32)
        row = 2 * lax.broadcasted_iota(I32, q.shape, 0)
        q = jnp.where(((row - h * DH) & (LANES - 1)) < DH, q, 0)
        return pltpu.bitcast(q, BF16)

    def head_v(h):
        base = pl.multiple_of((h * DH) & -8, 8)
        vt = jnp.concatenate(
            [vt_v[r, pl.ds(base, VR), :] for r in range(NB)], axis=1)
        row = lax.broadcasted_iota(I32, vt.shape, 0) - (h * DH - base)
        ones = jnp.where((row < 0) | (row >= DH), 1.0, vt)
        return jnp.concatenate([ones[:8], vt[8:VR - 8], ones[VR - 8:]], axis=0)

    def row_max(h, g):
        m = m_v[g, 0:1, :]
        return jnp.maximum(m, mx_v[h, g, 0:1, :]) if NX else m

    def probs(h, g, c, m):
        if NU <= c < NU + NX:
            s = jnp.concatenate(
                [s_v[g, pl.ds(c * CK, CK - UK), :],
                 sx_v[h, g, pl.ds((c - NU) * UK, UK), :]], axis=0)
        else:
            s = s_v[g, pl.ds(c * CK, CK), :]
        p = jnp.exp2(s - m)
        return p if PF32 else p.astype(BF16)

    def finish(h, g, acc):
        base = pl.multiple_of((h * DH) & -8, 8)
        shifted = h * DH - base
        total = jnp.where(shifted > 0, acc[:1], acc[VR - 1:])
        o = acc * (1.0 / total)
        row = lax.broadcasted_iota(I32, (8, RB), 0)
        first = jnp.where(row < shifted, ot_v[g, pl.ds(base, 8), :], o[:8])
        ot_v[g, pl.ds(base, VR), :] = jnp.concatenate([first, o[8:]], axis=0)

    def step(nxt, cur, units, jobs=()):
        on_mxu = [CK - UK if c < units or NU <= c < NU + NX else CK
                  for c in range(NC)]
        rows = sum(on_mxu) + (0 if cur is None else NC * VR)
        bg = _Background(never(), NB * rows // 8, LEAD)
        bg.jobs += jobs
        m = [None] * NB
        ready = []
        k = kw_v[window(nxt)]
        if units:
            qf_v[0] = qh_v[nxt]
            ku = [to_lane0(k[(u + 1) * CK - UK:(u + 1) * CK], nxt)
                  for u in range(units)]
        for g in range(NB):
            for u in range(units):
                def emit(s, g=g, u=u):
                    m[g] = _fold_max(m[g], s)
                    ready.append((g, u, s))
                bg.jobs += _score_jobs(ku[u], qf_v.at[0, g], emit)

        def store_ready(g, c):
            while ready and ready[0][:2] <= (g, c):
                gs, u, s = ready.pop(0)
                s_v[gs, unit_keys(u), :] = s

        if cur is not None:
            vt = head_v(cur)
        for g in range(NB):
            q = head_q(nxt, g)
            if cur is not None:
                m_cur = row_max(cur, g)
                acc = z_v[...]
            for c in range(NC):
                s = _dot(k[c * CK:c * CK + on_mxu[c]], q)
                m[g] = _fold_max(m[g], s)
                bg.tick(s)
                if cur is not None:
                    o = _dot(vt[:, c * CK:(c + 1) * CK], probs(cur, g, c, m_cur))
                    acc = acc + o
                    bg.tick(o)
                s_v[g, pl.ds(c * CK, on_mxu[c]), :] = s
                bg.run()
                store_ready(g, c)
            if cur is not None:
                finish(cur, g, acc)
        bg.run(last=True)
        store_ready(NB, NC)
        for g in range(NB):
            m_v[g] = jnp.broadcast_to(
                jnp.max(m[g], axis=0, keepdims=True), (8, RB))

    for c in w_copies:
        c.wait()
    with scope("ph2_qk0"):
        step(0, None, NU0,
             _strassen_rhs_jobs(wg_v, sg_v)
             + _strassen_rhs_jobs(wu_v, su_v)
             + _strassen_rhs_jobs(wd_v, sd_v))

    def ffn(r):
        rows = pl.ds(pl.multiple_of(r * RB, RB), RB)
        W1, W2, W3 = 0.5, 0.5, 0.75
        shares = ([1, 1, 1, 1, 1, 1, 1, W3] + [1, 1, 1, W3, W1, W1, W1, W1]) * 3
        shares += [1] * 14 + [W3, W3] + [1, 1, W2, W2, W2, W2, W2, W2]
        bg = _Background(never(), sum(
            round(32 * (1 if i % 8 else 2) * w) for i, w in enumerate(shares)), XLEAD)
        shares = iter(shares)
        for i in range(H // NB if NX else 0):
            h = r * (H // NB) + i
            qf_v[i] = qh_v[h]
            ku = [to_lane0(kw_v[window(h), unit_keys(NU + u), :], h)
                  for u in range(NX)]
            for g in range(NB):
                got = []
                for u in range(NX):
                    def emit(s, h=h, g=g, u=u, got=got):
                        sx_v[h, g, pl.ds(u * UK, UK), :] = s
                        got.append(_fold_max(got[-1] if got else None, s))
                        if u == NX - 1:
                            mx_v[h, g] = jnp.broadcast_to(jnp.max(
                                got[-1], axis=0, keepdims=True), (8, RB))
                    bg.jobs += _score_jobs(ku[u], qf_v.at[i, g], emit)

        def dot(a, w):
            out = _dot(a, w)
            bg.tick(out, next(shares))
            bg.run()
            return out

        def quadrants(a):
            return [a[i:i + RB // 2, j:j + KH]
                    for i in (0, RB // 2) for j in (0, KH)]

        xn = xn_v[rows, :]
        lhs = _strassen_lhs(*quadrants(xn))
        half = wd_v.shape[0] // 2

        def up(w_ref, sums_ref, j):
            w = jnp.concatenate([w_ref[2 * KH:, j:j + KH],
                                 w_ref[2 * KH:, half + j:half + j + KH]], axis=1)
            return dot(xn[:, 2 * KH:], w) + _strassen_combine(
                *_strassen(lhs, w_ref, sums_ref, 0, j, dot))

        hid = []
        for j in range(0, half, KH):
            g = 0.5 * up(wg_v, sg_v, j)
            hid.append(g * (1.0 + jnp.tanh(g)) * up(wu_v, su_v, j))
        parts = None
        for j, hj in zip(range(0, half, KH), hid):
            w = jnp.concatenate([wd_v[j:j + KH, 2 * KH:],
                                 wd_v[half + j:half + j + KH, 2 * KH:]], axis=0)
            new = [dot(hj.astype(BF16), w)] + _strassen(
                _strassen_lhs(*quadrants(hj)), wd_v, sd_v, j, 0, dot)
            parts = new if parts is None else [
                p + q for p, q in zip(parts, new)]
        y = jnp.concatenate([_strassen_combine(*parts[1:]), parts[0]], axis=1)
        bg.run(last=True)
        y_v[rows, :] = x_v[rows, :].astype(F32) + y

    with scope("ph3_ffn"):
        loop(0, NB, ffn)

    with scope("ph4_attn"):
        loop(0, H - 1, lambda h: step(h + 1, h, NU))

    vt = head_v(H - 1)

    def last_head(g, fillers):
        m = row_max(H - 1, g)
        acc = z_v[...]
        out = []
        for i, filler in enumerate(fillers):
            out.append(filler())
            for c in range(i * NC // len(fillers), (i + 1) * NC // len(fillers)):
                acc = acc + _dot(vt[:, c * CK:(c + 1) * CK], probs(H - 1, g, c, m))
        finish(H - 1, g, acc)
        return out

    def o_rows(g, lo, hi):
        return ot_v[g, lo:hi, :].astype(BF16).T

    def write(g, y):
        rows = pl.ds(g * RB, RB)
        out_v[rows, :] = (y_v[rows, :] + y).astype(out_v.dtype)

    def o_tile(g, t):
        lo = t * LANES
        return lambda: _dot(o_rows(g, lo, lo + LANES), wo_v[lo:lo + LANES, :])

    with scope("ph5_out"):
        y0 = last_head(0, [o_tile(0, 0), o_tile(0, 1)])
        y0 += last_head(1, [o_tile(0, 2), o_tile(0, 3)])
        y1 = last_head(2, [o_tile(0, 4), o_tile(1, 0)])
        write(0, sum(y0[1:], y0[0]) + y1[0])
        y1 = y1[1:] + last_head(3, [o_tile(1, 1), o_tile(1, 2)])
        y1 += [o_tile(1, 3)(), o_tile(1, 4)()]
        write(1, sum(y1[1:], y1[0]))
        xn_v[:RB, :] = o_rows(2, 0, D)
        out_copy(0).start()
        out_copy(1).start()
        write(2, _dot(xn_v[:RB, :], wo_v[...]))
        xn_v[RB:2 * RB, :] = o_rows(3, 0, D)
        out_copy(2).start()
        write(3, _dot(xn_v[RB:2 * RB, :], wo_v[...]))
        out_copy(3).start()
    with scope("ph6_wait"):
        for r in range(NB):
            out_copy(r).wait()


@jax.jit
def pallas_parallel_sum__mha_block__swiglu_ffn__prompt_kernel(
    A_x: jax.Array,
    A_wqkv: jax.Array,
    A_wo: jax.Array,
    B_x: jax.Array,
    B_w_gate: jax.Array,
    B_w_up: jax.Array,
    B_w_down: jax.Array,
):
    del B_x
    B, S, D = A_x.shape
    F = B_w_gate.shape[1]
    assert (B, S, D) == (1, 2048, 20 * H)
    weights = (A_wqkv, A_wo, B_w_gate, B_w_up, B_w_down)
    nb = S // RB
    any_spec = pl.BlockSpec(memory_space=pl.ANY)
    out = pl.pallas_call(
        _kernel,
        out_shape=jax.ShapeDtypeStruct((S, D), A_x.dtype),
        in_specs=[any_spec] * 6,
        out_specs=any_spec,
        scratch_shapes=[
            pltpu.VMEM((S, D), A_x.dtype),
            *[pltpu.VMEM(w.shape, w.dtype) for w in weights],
            pltpu.VMEM((S, D), BF16),
            pltpu.VMEM((2 * D, D), BF16),
            pltpu.VMEM((2 * (D // LANES) - 1, S, LANES), BF16),
            pltpu.VMEM((nb, D, RB), BF16),
            pltpu.VMEM((H, nb, D // H, RB), F32),
            pltpu.VMEM((H // nb, nb, D // H, RB), F32),
            pltpu.VMEM((nb, D, RB), F32),
            pltpu.VMEM((nb, D, RB), F32),
            pltpu.VMEM((nb, S, RB), F32),
            pltpu.VMEM((nb, 8, RB), F32),
            pltpu.VMEM((H, nb, max(NX, 1) * UK, RB), F32),
            pltpu.VMEM((H, nb, 8, RB), F32),
            pltpu.VMEM((VR, RB), F32),
            pltpu.VMEM((5, KH, F // 2), BF16),
            pltpu.VMEM((5, KH, F // 2), BF16),
            pltpu.VMEM((5, F // 2, KH), BF16),
            pltpu.VMEM((S, D), F32),
            pltpu.VMEM((S, D), A_x.dtype),
            pltpu.SemaphoreType.DMA((nb,)),
            pltpu.SemaphoreType.DMA((3,)),
            pltpu.SemaphoreType.DMA((4,)),
            pltpu.SemaphoreType.DMA((nb,)),
        ],
        compiler_params=pltpu.CompilerParams(
            vmem_limit_bytes=120 * 1024 * 1024),
        name="mha_swiglu_parallel",
    )(A_x.reshape(S, D), *weights)
    return out.reshape(B, S, D)
```

```python
import math

import jax
import jax.numpy as jnp
from jax import lax
from jax.experimental import pallas as pl
from jax.experimental.pallas import tpu as pltpu

H = 32
EPS = 1e-5
LANES = 128
RB = 512
CK = 128
UK = 16
NU = 12
NX = 4
VR = 24
KH = 256
X_CUTS = (0, 256, 640, 1024, 1536, 2048)
OUT_CUTS = (0, 512, 1024, 1664, 2048)

F32 = jnp.float32
BF16 = jnp.bfloat16
I32 = jnp.int32


def _dot(a, b, dims=((1,), (0,))):
    return lax.dot_general(a, b, (dims, ((), ())), preferred_element_type=F32)


def _lane_gather(x, idx):
    return lax.gather(
        x, idx[..., None],
        lax.GatherDimensionNumbers(
            offset_dims=(), collapsed_slice_dims=(1,), start_index_map=(1,),
            operand_batching_dims=(0,), start_indices_batching_dims=(0,)),
        slice_sizes=(1, 1), mode=lax.GatherScatterMode.PROMISE_IN_BOUNDS)


def _fold_max(m, s):
    s = jnp.max(s.reshape(-1, 8, s.shape[-1]), axis=0)
    return s if m is None else jnp.maximum(m, s)


def _column_max(m):
    return jnp.broadcast_to(jnp.max(m, axis=0, keepdims=True), m.shape)


class _Background:
    def __init__(self, zero_ref, n_ticks, lead):
        self.zero = pltpu.bitcast(zero_ref[:8, :LANES], I32)
        self.n_ticks, self.lead = n_ticks, lead
        self.jobs, self.ticks, self.done = [], [], 0

    def tick(self, result, share=1.0):
        n = result.shape[0] // 8
        keep = round(n * share)
        self.ticks += [result[8 * (i * n // keep):][:8, :LANES]
                       for i in range(keep)]

    def run(self, last=False):
        while self.done < len(self.jobs):
            t = self.done * self.n_ticks // len(self.jobs) - self.lead
            if t >= len(self.ticks) and not last:
                break

            def after(x):
                if not 0 <= t < len(self.ticks):
                    return x
                reps = (x.shape[0] // 8, x.shape[1] // LANES)
                tick = pltpu.bitcast(self.ticks[t], I32)
                return jnp.where(
                    jnp.tile(self.zero, reps) != 0, jnp.tile(tick, reps), x)

            self.jobs[self.done](after)
            self.done += 1

    def dot_by_tiles(self, a, b, dims):
        out = None
        for a_tile, b_tile in zip(a, b):
            part = _dot(a_tile, b_tile, dims)
            out = part if out is None else out + part
            self.tick(part)
            self.run()
        return out


def _score_jobs(k, q_ref, emit):
    dh, nq = q_ref.shape
    acc = []

    def job(d, after):
        idx = after(jnp.full((8, LANES), d, I32))
        kd = [_lane_gather(k[a:a + 8], idx) for a in range(0, UK, 8)]
        qd = [q_ref[d:d + 1, j:j + LANES] for j in range(0, nq, LANES)]
        new = [[ka * qj for qj in qd] for ka in kd]
        acc[:] = new if d == 0 else [
            [x + y for x, y in zip(xs, ys)] for xs, ys in zip(acc, new)]
        if d == dh - 1:
            emit(jnp.concatenate(
                [jnp.concatenate(xs, axis=1) for xs in acc], axis=0))

    return [lambda after, d=d: job(d, after) for d in range(dh)]


def _strassen_rhs_jobs(w_ref, sums_ref):
    _, k, n = sums_ref.shape

    def job(row, col, after):
        b11, b12, b21, b22 = (
            pltpu.bitcast(after(pltpu.bitcast(
                w_ref[pl.ds(i * k + row, 16), pl.ds(j * n + col, KH)], I32)),
                BF16).astype(F32)
            for i in range(2) for j in range(2))
        for i, b in enumerate(
                (b11 + b22, b12 - b22, b21 - b11, b11 + b12, b21 + b22)):
            sums_ref[i, pl.ds(row, 16), pl.ds(col, KH)] = b.astype(BF16)

    return [lambda after, row=row, col=col: job(row, col, after)
            for row in range(0, k, 16) for col in range(0, n, KH)]


def _strassen_lhs(a):
    m = a.shape[0] // 2
    a11, a12, a21, a22 = (
        a[i:i + m, j:j + KH] for i in (0, m) for j in (0, KH))
    f11, f12, f21, f22 = (t.astype(F32) for t in (a11, a12, a21, a22))
    return [t.astype(BF16) for t in (
        f11 + f22, f21 + f22, a11, a22, f11 + f12, f21 - f11, f12 - f22)]


def _strassen_products(lhs, w_ref, sums_ref, i, j, dot):
    _, k, n = sums_ref.shape
    rows, cols = pl.ds(i, KH), pl.ds(j, KH)
    return [
        dot(lhs[0], sums_ref[0, rows, cols]),
        dot(lhs[1], w_ref[rows, cols]),
        dot(lhs[2], sums_ref[1, rows, cols]),
        dot(lhs[3], sums_ref[2, rows, cols]),
        dot(lhs[4], w_ref[pl.ds(k + i, KH), pl.ds(n + j, KH)]),
        dot(lhs[5], sums_ref[3, rows, cols]),
        dot(lhs[6], sums_ref[4, rows, cols]),
    ]


def _strassen_combine(m1, m2, m3, m4, m5, m6, m7):
    return jnp.concatenate(
        [jnp.concatenate([m1 + m4 - m5 + m7, m3 + m5], axis=1),
         jnp.concatenate([m2 + m4, m1 - m2 + m3 + m6], axis=1)], axis=0)


def _kernel(
    x_hbm, wqkv_hbm, wo_hbm, wg_hbm, wu_hbm, wd_hbm,
    out_hbm,
    x_v, wqkv_v, wo_v, wg_v, wu_v, wd_v,
    xn_v, wt_v, k_v, kh_v, qh_v, qf_v, vt_v, ot_v,
    s_v, m_v, sx_v, mx_v, z_v, acc_v,
    sg_v, su_v, sd_v, y_v, out_v,
    x_sem, qkv_sem, w_sem, out_sem,
):
    S, D = x_v.shape
    DH = D // H
    NT = D // LANES
    NB = S // RB
    NC = S // CK
    tiles = [pl.ds(i, LANES) for i in range(0, D, LANES)]

    def row_copy(src, dst, sem, cuts, i):
        rows = pl.ds(cuts[i], cuts[i + 1] - cuts[i])
        return pltpu.make_async_copy(src.at[rows], dst.at[rows], sem.at[i])

    x_copies = [row_copy(x_hbm, x_v, x_sem, X_CUTS, i)
                for i in range(len(X_CUTS) - 1)]
    out_copies = [row_copy(out_v, out_hbm, out_sem, OUT_CUTS, i)
                  for i in range(len(OUT_CUTS) - 1)]
    wq_copy, wk_copy, wv_copy = (
        pltpu.make_async_copy(
            wqkv_hbm.at[:, pl.ds(i * D, D)], wqkv_v.at[i], qkv_sem.at[i])
        for i in range(3))
    w_copies = [
        pltpu.make_async_copy(src, dst, w_sem.at[i])
        for i, (src, dst) in enumerate(
            [(wo_hbm, wo_v), (wg_hbm, wg_v), (wu_hbm, wu_v), (wd_hbm, wd_v)])
    ]

    def loop(n, body):
        def step(i, carry):
            body(i)
            return carry
        lax.fori_loop(0, n, step, None)

    def block(r):
        return pl.ds(pl.multiple_of(r * RB, RB), RB)

    def lane_tiles(a):
        return (a[:, i:i + LANES] for i in range(0, D, LANES))

    def layernorm(lo, n, after=lambda x: x):
        rows = pl.ds(lo, n)
        x = pltpu.bitcast(
            after(pltpu.bitcast(x_v[rows, :], I32)), BF16).astype(F32)
        xc = x - jnp.mean(x, axis=-1, keepdims=True)
        var = jnp.mean(xc * xc, axis=-1, keepdims=True)
        xn_v[rows, :] = (xc * lax.rsqrt(var + EPS)).astype(BF16)

    def project_k(lo, hi, norm_hi):
        xn = xn_v[lo:hi, :]
        bg = _Background(z_v, (NT - 1) * (hi - lo) // 8, 0)
        bg.jobs += [lambda after, i=i: layernorm(i, 16, after)
                    for i in range(hi, norm_hi, 16)]
        k = bg.dot_by_tiles(
            lane_tiles(xn), (wqkv_v[1, t, :D - LANES] for t in tiles),
            ((1,), (0,)))
        bg.run(last=True)
        k = jnp.concatenate([k, _dot(xn, wqkv_v[1, :, D - LANES:])], axis=1)
        k_v[lo:hi, :] = k.astype(BF16)

    def project_q(r):
        def split_keys(lo, first, after):
            rows = pl.ds(pl.multiple_of(r * RB + lo, 16), 16)
            words = pl.ds(pl.multiple_of(r * (RB // 2) + lo // 2, 8), 8)
            k = after(pltpu.bitcast(k_v[rows, first:first + LANES], I32))
            for h in range(-(-first // DH), -(-(first + LANES) // DH)):
                if (h + 1) * DH > first + LANES:
                    lane = lax.broadcasted_iota(I32, k.shape, 1)
                    k = jnp.where(lane < DH, pltpu.bitcast(
                        k_v[rows, first + LANES:first + 2 * LANES], I32), k)
                shift = (first - h * DH) % LANES
                kh_v[h, words, :] = pltpu.roll(k, shift, 1) if shift else k

        bg = _Background(z_v, NT * D // 8, 20)
        bg.jobs += [lambda after, lo=lo, i=i: split_keys(lo, i, after)
                    for lo in range(0, RB, 16) for i in range(0, D, LANES)]
        qt = bg.dot_by_tiles(
            (wt_v[0, :, t] for t in tiles), lane_tiles(xn_v[block(r), :]),
            ((1,), (1,)))
        bg.run(last=True)
        qt = qt * (DH ** -0.5 * math.log2(math.e))
        qt = qt.astype(BF16).astype(F32)
        for h in range(H):
            qh_v[h, r] = qt[h * DH:(h + 1) * DH]

    x_copies[0].start()
    wk_copy.start()
    x_copies[1].start()
    z_v[...] = jnp.zeros_like(z_v)
    acc_v[...] = jnp.ones_like(acc_v)
    x_copies[0].wait()
    layernorm(0, 256)
    wk_copy.wait()
    x_copies[1].wait()
    x_copies[2].start()
    x_copies[3].start()
    project_k(0, 256, 512)
    project_k(256, 512, 640)
    x_copies[2].wait()
    x_copies[3].wait()
    x_copies[4].start()
    wq_copy.start()
    wv_copy.start()
    project_k(512, 640, 896)
    project_k(640, 896, 1408)
    project_k(896, 1408, 1536)
    x_copies[4].wait()
    wq_copy.wait()
    wv_copy.wait()
    for c in w_copies:
        c.start()
    project_k(1408, 1536, 1792)
    project_k(1536, 1792, 2048)
    project_k(1792, 2048, 2048)
    wt_v[0] = wqkv_v[0].T
    wt_v[1] = wqkv_v[2].T
    loop(NB // 2, lambda i: (project_q(2 * i), project_q(2 * i + 1)))

    def head_v(h):
        base = pl.multiple_of((h * DH) & -8, 8)
        vt = jnp.concatenate(
            [vt_v[r, pl.ds(base, VR), :] for r in range(NB)], axis=1)
        row = lax.broadcasted_iota(I32, vt.shape, 0) - (h * DH - base)
        ones = jnp.where((row < 0) | (row >= DH), 1.0, vt)
        return jnp.concatenate([ones[:8], vt[8:VR - 8], ones[VR - 8:]], axis=0)

    def row_max(h, g):
        return jnp.maximum(m_v[g, 0:1, :], mx_v[h, g, 0:1, :])

    def probs(h, g, c, m):
        if NU <= c < NU + NX:
            s = jnp.concatenate(
                [s_v[g, pl.ds(c * CK, CK - UK), :],
                 sx_v[h, g, pl.ds((c - NU) * UK, UK), :]], axis=0)
        else:
            s = s_v[g, pl.ds(c * CK, CK), :]
        return jnp.exp2(s - m)

    def finish(h, g, acc):
        base = pl.multiple_of((h * DH) & -8, 8)
        skip = h * DH - base
        total = jnp.where(skip > 0, acc[:1], acc[VR - 1:])
        o = acc * (1.0 / total)
        row = lax.broadcasted_iota(I32, (8, RB), 0)
        first = jnp.where(row < skip, ot_v[g, pl.ds(base, 8), :], o[:8])
        ot_v[g, pl.ds(base, VR), :] = jnp.concatenate([first, o[8:]], axis=0)

    def attend(nxt, cur, units, jobs=()):
        on_mxu = [CK - UK if c < units or NU <= c < NU + NX else CK
                  for c in range(NC)]
        rows = sum(on_mxu) + (0 if cur is None else NC * VR)
        bg = _Background(z_v, NB * rows // 8, 20)
        bg.jobs += jobs
        m = [None] * NB
        ready = []
        k = pltpu.bitcast(kh_v[nxt], BF16)
        q = qh_v[nxt]
        if units:
            qf_v[0] = q
        ku = [k[(u + 1) * CK - UK:(u + 1) * CK].astype(F32)
              for u in range(units)]
        k = k[:, :DH]
        for g in range(NB):
            for u in range(units):
                def emit(s, g=g, u=u):
                    m[g] = _fold_max(m[g], s)
                    ready.append((g, u, s))
                bg.jobs += _score_jobs(ku[u], qf_v.at[0, g], emit)

        def store_ready(g, c):
            while ready and ready[0][:2] <= (g, c):
                gs, u, s = ready.pop(0)
                s_v[gs, pl.ds((u + 1) * CK - UK, UK), :] = s

        if cur is not None:
            vt = head_v(cur)
        for g in range(NB):
            if cur is not None:
                m_cur = row_max(cur, g)
                acc = z_v[...]
            for c in range(NC):
                s = _dot(k[c * CK:c * CK + on_mxu[c]], q[g])
                m[g] = _fold_max(m[g], s)
                bg.tick(s)
                if cur is not None:
                    o = _dot(vt[:, c * CK:(c + 1) * CK],
                             probs(cur, g, c, m_cur))
                    acc = acc + o
                    bg.tick(o)
                s_v[g, pl.ds(c * CK, on_mxu[c]), :] = s
                bg.run()
                store_ready(g, c)
            if cur is None:
                continue
            if g == NB - 1:
                acc_v[...] = acc
            else:
                finish(cur, g, acc)
            if g == 0:
                finish(jnp.maximum(cur - 1, 0), NB - 1, acc_v[...])
        bg.run(last=True)
        store_ready(NB, NC)
        for g in range(NB):
            m_v[g] = _column_max(m[g])

    for c in w_copies:
        c.wait()
    attend(0, None, 0,
           _strassen_rhs_jobs(wg_v, sg_v) + _strassen_rhs_jobs(wu_v, su_v)
           + _strassen_rhs_jobs(wd_v, sd_v))

    def swiglu(r):
        shares = ([1, 1, 1, 1, 1, .75, .75, .4]
                  + [1, 1, 1, .75, .4, .4, .4, .4]) * 3
        shares[4:8] = [.75, .4, .4, .4]
        shares += [1] * 14 + [.75, .75, 1, 1] + [.4] * 6
        n_ticks = sum(round(RB // (16 if i % 8 else 8) * w)
                      for i, w in enumerate(shares))
        bg = _Background(z_v, NT * D // 8 + n_ticks, 12)
        shares = iter(shares)
        for i in range(H // NB):
            h = r * (H // NB) + i
            qf_v[i] = qh_v[h]
            ku = [pltpu.bitcast(
                kh_v[h, pl.ds(((NU + u + 1) * CK - UK) // 2, UK // 2), :],
                BF16).astype(F32) for u in range(NX)]
            for g in range(NB):
                m = [None]
                for u in range(NX):
                    def emit(s, h=h, g=g, u=u, m=m):
                        sx_v[h, g, pl.ds(u * UK, UK), :] = s
                        m[0] = _fold_max(m[0], s)
                        if u == NX - 1:
                            mx_v[h, g] = _column_max(m[0])
                    bg.jobs += _score_jobs(ku[u], qf_v.at[i, g], emit)

        def dot(a, w):
            out = _dot(a, w)
            bg.tick(out, next(shares))
            bg.run()
            return out

        xn = xn_v[block(r), :]
        vt_v[r] = bg.dot_by_tiles(
            (wt_v[1, :, t] for t in tiles), lane_tiles(xn), ((1,), (1,)))
        lhs = _strassen_lhs(xn)
        half = wd_v.shape[0] // 2

        def up(w_ref, sums_ref, j):
            w = jnp.concatenate(
                [w_ref[2 * KH:, j:j + KH],
                 w_ref[2 * KH:, half + j:half + j + KH]], axis=1)
            return dot(xn[:, 2 * KH:], w) + _strassen_combine(
                *_strassen_products(lhs, w_ref, sums_ref, 0, j, dot))

        hid = []
        for j in range(0, half, KH):
            g = 0.5 * up(wg_v, sg_v, j)
            hid.append(g * (1.0 + jnp.tanh(g)) * up(wu_v, su_v, j))
        parts = None
        for j, hj in zip(range(0, half, KH), hid):
            w = jnp.concatenate(
                [wd_v[j:j + KH, 2 * KH:],
                 wd_v[half + j:half + j + KH, 2 * KH:]], axis=0)
            new = [dot(hj.astype(BF16), w)] + _strassen_products(
                _strassen_lhs(hj), wd_v, sd_v, j, 0, dot)
            parts = new if parts is None else [
                a + b for a, b in zip(parts, new)]
        y = jnp.concatenate([_strassen_combine(*parts[1:]), parts[0]], axis=1)
        bg.run(last=True)
        y_v[block(r), :] = x_v[block(r), :].astype(F32) + y

    loop(NB, swiglu)
    loop(H - 1, lambda h: attend(h + 1, h, NU))

    vt = head_v(H - 1)

    def o_rows(g, lo, hi):
        return ot_v[g, lo:hi, :].astype(BF16).T

    def o_tile(g, t):
        return _dot(o_rows(g, t * LANES, (t + 1) * LANES), wo_v[tiles[t], :])

    def last_head(g, done):
        m = row_max(H - 1, g)
        acc = z_v[...]
        out = []
        for i, tile in enumerate(done):
            out.append(o_tile(*tile))
            for c in range(i * NC // len(done), (i + 1) * NC // len(done)):
                acc = acc + _dot(
                    vt[:, c * CK:(c + 1) * CK], probs(H - 1, g, c, m))
        finish(H - 1, g, acc)
        return out

    def write(lo, y):
        rows = pl.ds(lo, y.shape[0])
        out_v[rows, :] = (y_v[rows, :] + y).astype(out_v.dtype)

    finish(H - 2, NB - 1, acc_v[...])
    y0 = last_head(0, [(0, 0), (0, 1)]) + last_head(1, [(0, 2), (0, 3)])
    y1 = last_head(2, [(0, 4), (1, 0)])
    write(0, sum(y0[1:], y0[0]) + y1[0])
    y1 = y1[1:] + last_head(3, [(1, 1), (1, 2)]) + [o_tile(1, 3), o_tile(1, 4)]
    write(RB, sum(y1[1:], y1[0]))
    xn_v[:RB, :] = o_rows(2, 0, D)
    out_copies[0].start()
    out_copies[1].start()
    write(2 * RB, _dot(xn_v[:RB, :], wo_v[...]))
    cut = OUT_CUTS[3] - 3 * RB
    o3 = o_rows(3, 0, D)
    write(3 * RB, _dot(o3[:cut], wo_v[...]))
    xn_v[RB:2 * RB - cut, :] = o3[cut:]
    out_copies[2].start()
    write(OUT_CUTS[3], _dot(xn_v[RB:2 * RB - cut, :], wo_v[...]))
    out_copies[3].start()
    for c in out_copies:
        c.wait()


@jax.jit
def pallas_parallel_sum__mha_block__swiglu_ffn__prompt_kernel(
    A_x: jax.Array,
    A_wqkv: jax.Array,
    A_wo: jax.Array,
    B_x: jax.Array,
    B_w_gate: jax.Array,
    B_w_up: jax.Array,
    B_w_down: jax.Array,
):
    del B_x
    B, S, D = A_x.shape
    F = B_w_gate.shape[1]
    assert (B, S, D, F) == (1, 2048, 640, 1536) and A_x.dtype == BF16
    weights = (A_wqkv, A_wo, B_w_gate, B_w_up, B_w_down)
    nb = S // RB
    any_spec = pl.BlockSpec(memory_space=pl.ANY)
    out = pl.pallas_call(
        _kernel,
        out_shape=jax.ShapeDtypeStruct((S, D), A_x.dtype),
        in_specs=[any_spec] * 6,
        out_specs=any_spec,
        scratch_shapes=[
            pltpu.VMEM((S, D), A_x.dtype),
            pltpu.VMEM((3, D, D), A_wqkv.dtype),
            *[pltpu.VMEM(w.shape, w.dtype) for w in weights[1:]],
            pltpu.VMEM((S, D), BF16),
            pltpu.VMEM((2, D, D), BF16),
            pltpu.VMEM((S, D), BF16),
            pltpu.VMEM((H, S // 2, LANES), I32),
            pltpu.VMEM((H, nb, D // H, RB), F32),
            pltpu.VMEM((H // nb, nb, D // H, RB), F32),
            pltpu.VMEM((nb, D, RB), F32),
            pltpu.VMEM((nb, D, RB), F32),
            pltpu.VMEM((nb, S, RB), F32),
            pltpu.VMEM((nb, 8, RB), F32),
            pltpu.VMEM((H, nb, NX * UK, RB), F32),
            pltpu.VMEM((H, nb, 8, RB), F32),
            pltpu.VMEM((VR, RB), F32),
            pltpu.VMEM((VR, RB), F32),
            pltpu.VMEM((5, KH, F // 2), BF16),
            pltpu.VMEM((5, KH, F // 2), BF16),
            pltpu.VMEM((5, F // 2, KH), BF16),
            pltpu.VMEM((S, D), F32),
            pltpu.VMEM((S, D), A_x.dtype),
            pltpu.SemaphoreType.DMA((len(X_CUTS) - 1,)),
            pltpu.SemaphoreType.DMA((3,)),
            pltpu.SemaphoreType.DMA((4,)),
            pltpu.SemaphoreType.DMA((len(OUT_CUTS) - 1,)),
        ],
        compiler_params=pltpu.CompilerParams(
            vmem_limit_bytes=120 * 1024 * 1024),
        name="mha_swiglu_parallel",
    )(A_x.reshape(S, D), *weights)
    return out.reshape(B, S, D)
```

```python
import math

import jax
import jax.numpy as jnp
from jax import lax
from jax.experimental import pallas as pl
from jax.experimental.pallas import tpu as pltpu

H = 32
EPS = 1e-5
LANES = 128
QUAD = 4 * LANES
RB = 512
CK = 128
UK = 16
NU = 12
NX = 6
UNIT_CHUNKS = (*range(16), 4, 13)
VR = 24
X_CUTS = (0, 256, 640, 1024, 1536, 2048)
OUT_CUTS = (0, 512, 1024, 1664, 2048)

F32 = jnp.float32
BF16 = jnp.bfloat16
I32 = jnp.int32


def _dot(a, b, dims=((1,), (0,))):
    return lax.dot_general(a, b, (dims, ((), ())), preferred_element_type=F32)


def _lane_gather(x, idx):
    return lax.gather(
        x, idx[..., None],
        lax.GatherDimensionNumbers(
            offset_dims=(), collapsed_slice_dims=(1,), start_index_map=(1,),
            operand_batching_dims=(0,), start_indices_batching_dims=(0,)),
        slice_sizes=(1, 1), mode=lax.GatherScatterMode.PROMISE_IN_BOUNDS)


def _fold_max(m, s):
    s = jnp.max(s.reshape(-1, 8, s.shape[-1]), axis=0)
    return s if m is None else jnp.maximum(m, s)


def _column_max(m):
    return jnp.broadcast_to(jnp.max(m, axis=0, keepdims=True), m.shape)


class _Background:
    def __init__(self, zero_ref, n_ticks, lead):
        self.zero = pltpu.bitcast(zero_ref[:8, :LANES], I32)
        self.n_ticks, self.lead = n_ticks, lead
        self.jobs, self.ticks, self.done = [], [], 0

    def tick(self, result, share=1.0):
        n = result.shape[0] // 8
        keep = round(n * share)
        self.ticks += [result[8 * (i * n // keep):][:8, :LANES]
                       for i in range(keep)]

    def run(self, last=False):
        while self.done < len(self.jobs):
            t = self.done * self.n_ticks // len(self.jobs) - self.lead
            if t >= len(self.ticks) and not last:
                break

            def after(x):
                if not 0 <= t < len(self.ticks):
                    return x
                reps = (x.shape[0] // 8, x.shape[1] // LANES)
                tick = pltpu.bitcast(self.ticks[t], I32)
                return jnp.where(
                    jnp.tile(self.zero, reps) != 0, jnp.tile(tick, reps), x)

            self.jobs[self.done](after)
            self.done += 1

    def dot(self, a, b, n, dims=((1,), (0,)), share=1.0):
        def step(depths, columns):
            part = _dot(a[:, depths], b(depths, columns), dims)
            self.tick(part, share)
            self.run()
            return part

        depth = a.shape[1]
        full = depth // QUAD * QUAD
        rest = step(slice(full, depth), slice(0, n)) if full < depth else None
        out = []
        for j in range(0, n, LANES):
            acc = None if rest is None else rest[:, j:j + LANES]
            for i in range(0, full, QUAD):
                part = step(slice(i, i + QUAD), slice(j, j + LANES))
                acc = part if acc is None else acc + part
            out.append(acc)
        return jnp.concatenate(out, axis=1)


def _score_jobs(k, q_ref, emit):
    dh, nq = q_ref.shape
    acc = []

    def job(d, after):
        idx = after(jnp.full((8, LANES), d, I32))
        kd = [_lane_gather(k[a:a + 8], idx) for a in range(0, UK, 8)]
        qd = [q_ref[d:d + 1, j:j + LANES] for j in range(0, nq, LANES)]
        new = [[ka * qj for qj in qd] for ka in kd]
        acc[:] = new if d == 0 else [
            [x + y for x, y in zip(xs, ys)] for xs, ys in zip(acc, new)]
        if d == dh - 1:
            emit(jnp.concatenate(
                [jnp.concatenate(xs, axis=1) for xs in acc], axis=0))

    return [lambda after, d=d: job(d, after) for d in range(dh)]


def _kernel(
    x_hbm, wqkv_hbm, wo_hbm, wg_hbm, wu_hbm, wd_hbm,
    out_hbm,
    x_v, wqkv_v, wo_v, wg_v, wu_v, wd_v,
    xn_v, wt_v, k_v, kh_v, qh_v, qf_v, vt_v, ot_v,
    s_v, m_v, sx_v, mx_v, z_v, acc_v,
    y_v, out_v,
    x_sem, qkv_sem, w_sem, out_sem,
):
    S, D = x_v.shape
    DH = D // H
    NT = D // LANES
    NB = S // RB
    NC = S // CK

    def row_copy(src, dst, sem, cuts, i):
        rows = pl.ds(cuts[i], cuts[i + 1] - cuts[i])
        return pltpu.make_async_copy(src.at[rows], dst.at[rows], sem.at[i])

    x_copies = [row_copy(x_hbm, x_v, x_sem, X_CUTS, i)
                for i in range(len(X_CUTS) - 1)]
    out_copies = [row_copy(out_v, out_hbm, out_sem, OUT_CUTS, i)
                  for i in range(len(OUT_CUTS) - 1)]
    wq_copy, wk_copy, wv_copy = (
        pltpu.make_async_copy(
            wqkv_hbm.at[:, pl.ds(i * D, D)], wqkv_v.at[i], qkv_sem.at[i])
        for i in range(3))
    w_copies = [
        pltpu.make_async_copy(src, dst, w_sem.at[i])
        for i, (src, dst) in enumerate(
            [(wo_hbm, wo_v), (wg_hbm, wg_v), (wu_hbm, wu_v), (wd_hbm, wd_v)])
    ]

    def loop(n, body):
        def step(i, carry):
            body(i)
            return carry
        lax.fori_loop(0, n, step, None)

    def block(r):
        return pl.ds(pl.multiple_of(r * RB, RB), RB)

    def layernorm(lo, n, after=lambda x: x):
        rows = pl.ds(lo, n)
        x = pltpu.bitcast(
            after(pltpu.bitcast(x_v[rows, :], I32)), BF16).astype(F32)
        xc = x - jnp.mean(x, axis=-1, keepdims=True)
        var = jnp.mean(xc * xc, axis=-1, keepdims=True)
        xn_v[rows, :] = (xc * lax.rsqrt(var + EPS)).astype(BF16)

    def project_k(lo, hi, norm_hi):
        xn = xn_v[lo:hi, :]
        bg = _Background(z_v, (NT - 1) * (hi - lo) // 8, 0)
        bg.jobs += [lambda after, i=i: layernorm(i, 16, after)
                    for i in range(hi, norm_hi, 16)]
        k = bg.dot(xn, lambda i, j: wqkv_v[1, i, j], QUAD)
        bg.run(last=True)
        k = jnp.concatenate([k, _dot(xn, wqkv_v[1, :, QUAD:])], axis=1)
        k_v[lo:hi, :] = k.astype(BF16)

    def project_q(r):
        def split_keys(lo, first, after):
            rows = pl.ds(pl.multiple_of(r * RB + lo, 16), 16)
            words = pl.ds(pl.multiple_of(r * (RB // 2) + lo // 2, 8), 8)
            k = after(pltpu.bitcast(k_v[rows, first:first + LANES], I32))
            for h in range(-(-first // DH), -(-(first + LANES) // DH)):
                if (h + 1) * DH > first + LANES:
                    lane = lax.broadcasted_iota(I32, k.shape, 1)
                    k = jnp.where(lane < DH, pltpu.bitcast(
                        k_v[rows, first + LANES:first + 2 * LANES], I32), k)
                shift = (first - h * DH) % LANES
                kh_v[h, words, :] = pltpu.roll(k, shift, 1) if shift else k

        bg = _Background(z_v, NT * D // 8, 20)
        bg.jobs += [lambda after, lo=lo, i=i: split_keys(lo, i, after)
                    for lo in range(0, RB, 16) for i in range(0, D, LANES)]
        xn = xn_v[block(r), :]
        qt = bg.dot(wt_v[0], lambda i, j: xn[j, i], RB, ((1,), (1,)))
        bg.run(last=True)
        qt = qt * (DH ** -0.5 * math.log2(math.e))
        qt = qt.astype(BF16).astype(F32)
        for h in range(H):
            qh_v[h, r] = qt[h * DH:(h + 1) * DH]

    x_copies[0].start()
    wk_copy.start()
    x_copies[1].start()
    z_v[...] = jnp.zeros_like(z_v)
    ot_v[...] = jnp.zeros_like(ot_v)
    acc_v[...] = jnp.ones_like(acc_v)
    x_copies[0].wait()
    layernorm(0, 256)
    wk_copy.wait()
    x_copies[1].wait()
    x_copies[2].start()
    x_copies[3].start()
    project_k(0, 256, 512)
    project_k(256, 512, 640)
    x_copies[2].wait()
    x_copies[3].wait()
    x_copies[4].start()
    wq_copy.start()
    wv_copy.start()
    project_k(512, 640, 896)
    project_k(640, 896, 1280)
    project_k(896, 1280, 1536)
    x_copies[4].wait()
    wq_copy.wait()
    wv_copy.wait()
    for c in w_copies:
        c.start()
    project_k(1280, 1536, 1792)
    project_k(1536, 1792, 2048)
    project_k(1792, 2048, 2048)
    wt_v[0] = wqkv_v[0].T
    wt_v[1] = wqkv_v[2].T
    loop(NB // 2, lambda i: (project_q(2 * i), project_q(2 * i + 1)))

    def unit_start(u):
        return (UNIT_CHUNKS[u] + 1) * CK - (u // NC + 1) * UK

    on_mxu = [CK - UK * UNIT_CHUNKS.count(c) for c in range(NC)]

    def head_v(h):
        base = pl.multiple_of((h * DH) & -8, 8)
        vt = jnp.concatenate(
            [vt_v[r, pl.ds(base, VR), :] for r in range(NB)], axis=1)
        row = lax.broadcasted_iota(I32, vt.shape, 0) - (h * DH - base)
        ones = jnp.where((row < 0) | (row >= DH), 1.0, vt)
        return jnp.concatenate([ones[:8], vt[8:VR - 8], ones[VR - 8:]], axis=0)

    def row_max(h, g):
        return jnp.maximum(m_v[g, 0:1, :], mx_v[h, g, 0:1, :])

    def probs(h, g, c, m):
        s = [s_v[g, pl.ds(c * CK, on_mxu[c]), :]]
        for u in reversed(range(NU + NX)):
            if UNIT_CHUNKS[u] != c:
                continue
            s.append(s_v[g, pl.ds(unit_start(u), UK), :] if u < NU
                     else sx_v[h, g, pl.ds((u - NU) * UK, UK), :])
        s = jnp.concatenate(s, axis=0)
        return jnp.exp2(s - m)

    def finish(h, g, acc):
        base = pl.multiple_of((h * DH) & -8, 8)
        skip = h * DH - base
        total = jnp.where(skip > 0, acc[:1], acc[VR - 1:])
        o = acc * (1.0 / total)
        row = lax.broadcasted_iota(I32, (8, RB), 0)
        first = jnp.where(row < skip, ot_v[g, pl.ds(base, 8), :], o[:8])
        ot_v[g, pl.ds(base, VR), :] = jnp.concatenate([first, o[8:]], axis=0)

    def attend(nxt, cur):
        rows = sum(on_mxu) + (0 if cur is None else NC * VR)
        bg = _Background(z_v, NB * rows // 8, 20)
        m = [None] * NB
        ready = []
        k = pltpu.bitcast(kh_v[nxt], BF16)
        q = qh_v[nxt]
        qf_v[0] = q
        ku = [k[unit_start(u):unit_start(u) + UK].astype(F32)
              for u in range(NU)]
        k = k[:, :DH]
        for g in range(NB):
            for u in range(NU):
                def emit(s, g=g, u=u):
                    m[g] = _fold_max(m[g], s)
                    ready.append((g, u, s))
                bg.jobs += _score_jobs(ku[u], qf_v.at[0, g], emit)

        def store_ready(g, c):
            while ready and ready[0][:2] <= (g, c):
                gs, u, s = ready.pop(0)
                s_v[gs, pl.ds(unit_start(u), UK), :] = s

        if cur is not None:
            vt = head_v(cur)
        for g in range(NB):
            if cur is not None:
                m_cur = row_max(cur, g)
                acc = z_v[...]
            for c in range(NC):
                s = _dot(k[c * CK:c * CK + on_mxu[c]], q[g])
                m[g] = _fold_max(m[g], s)
                bg.tick(s)
                if cur is not None:
                    o = _dot(vt[:, c * CK:(c + 1) * CK],
                             probs(cur, g, c, m_cur))
                    acc = acc + o
                    bg.tick(o)
                s_v[g, pl.ds(c * CK, on_mxu[c]), :] = s
                bg.run()
                store_ready(g, c)
            if cur is None:
                continue
            if g == NB - 1:
                acc_v[...] = acc
            else:
                finish(cur, g, acc)
            if g == 0:
                finish(jnp.maximum(cur - 1, 0), NB - 1, acc_v[...])
        bg.run(last=True)
        store_ready(NB, NC)
        for g in range(NB):
            m_v[g] = _column_max(m[g])

    attend(0, None)
    for c in w_copies:
        c.wait()

    def swiglu(r):
        F = wd_v.shape[0]
        share = 13 / 16
        macs = round(RB * D * (D + (2 + share) * F))
        bg = _Background(z_v, macs // (8 * LANES * QUAD), 12)
        for i in range(H // NB):
            h = r * (H // NB) + i
            qf_v[i] = qh_v[h]
            ku = [pltpu.bitcast(
                kh_v[h, pl.ds(unit_start(NU + u) // 2, UK // 2), :],
                BF16).astype(F32) for u in range(NX)]
            for g in range(NB):
                m = [None]
                for u in range(NX):
                    def emit(s, h=h, g=g, u=u, m=m):
                        sx_v[h, g, pl.ds(u * UK, UK), :] = s
                        m[0] = _fold_max(m[0], s)
                        if u == NX - 1:
                            mx_v[h, g] = _column_max(m[0])
                    bg.jobs += _score_jobs(ku[u], qf_v.at[i, g], emit)

        xn = xn_v[block(r), :]
        hid = []
        for c in range(0, F, QUAD):
            wg, wu = wg_v.at[:, c:c + QUAD], wu_v.at[:, c:c + QUAD]
            g = bg.dot(xn, lambda i, j: wg[i, j], QUAD)
            u = bg.dot(xn, lambda i, j: wu[i, j], QUAD, share=share)
            g = 0.5 * g
            hid.append((g * (1.0 + jnp.tanh(g)) * u).astype(BF16))
        vt_v[r] = bg.dot(wt_v[1], lambda i, j: xn[j, i], RB, ((1,), (1,)))
        y = bg.dot(jnp.concatenate(hid, axis=1), lambda i, j: wd_v[i, j], D)
        bg.run(last=True)
        y_v[block(r), :] = x_v[block(r), :].astype(F32) + y

    loop(NB, swiglu)
    loop(H - 1, lambda h: attend(h + 1, h))

    vt = head_v(H - 1)

    def o_rows(g, lo, hi):
        return ot_v[g, lo:hi, :].astype(BF16).T

    def o_tile(g, t):
        lo, hi = t * LANES, (t + 1) * LANES
        return _dot(o_rows(g, lo, hi), wo_v[lo:hi, :])

    def last_head(g, done):
        m = row_max(H - 1, g)
        acc = z_v[...]
        out = []
        for i, tile in enumerate(done):
            out.append(o_tile(*tile))
            for c in range(i * NC // len(done), (i + 1) * NC // len(done)):
                acc = acc + _dot(
                    vt[:, c * CK:(c + 1) * CK], probs(H - 1, g, c, m))
        finish(H - 1, g, acc)
        return out

    def write(lo, y):
        rows = pl.ds(lo, y.shape[0])
        out_v[rows, :] = (y_v[rows, :] + y).astype(out_v.dtype)

    finish(H - 2, NB - 1, acc_v[...])
    y0 = last_head(0, [(0, 0), (0, 1)]) + last_head(1, [(0, 2), (0, 3)])
    y1 = last_head(2, [(0, 4), (1, 0)])
    write(0, sum(y0[1:], y0[0]) + y1[0])
    y1 = y1[1:] + last_head(3, [(1, 1), (1, 2)]) + [o_tile(1, 3), o_tile(1, 4)]
    write(RB, sum(y1[1:], y1[0]))
    xn_v[:RB, :] = o_rows(2, 0, D)
    out_copies[0].start()
    out_copies[1].start()
    write(2 * RB, _dot(xn_v[:RB, :], wo_v[...]))
    cut = OUT_CUTS[3] - 3 * RB
    o3 = o_rows(3, 0, D)
    write(3 * RB, _dot(o3[:cut], wo_v[...]))
    xn_v[RB:2 * RB - cut, :] = o3[cut:]
    out_copies[2].start()
    write(OUT_CUTS[3], _dot(xn_v[RB:2 * RB - cut, :], wo_v[...]))
    out_copies[3].start()
    for c in out_copies:
        c.wait()


@jax.jit
def pallas_parallel_sum__mha_block__swiglu_ffn__prompt_kernel(
    A_x: jax.Array,
    A_wqkv: jax.Array,
    A_wo: jax.Array,
    B_x: jax.Array,
    B_w_gate: jax.Array,
    B_w_up: jax.Array,
    B_w_down: jax.Array,
):
    del B_x
    B, S, D = A_x.shape
    F = B_w_gate.shape[1]
    assert (B, S, D, F) == (1, 2048, 640, 1536) and A_x.dtype == BF16
    weights = (A_wqkv, A_wo, B_w_gate, B_w_up, B_w_down)
    nb = S // RB
    any_spec = pl.BlockSpec(memory_space=pl.ANY)
    out = pl.pallas_call(
        _kernel,
        out_shape=jax.ShapeDtypeStruct((S, D), A_x.dtype),
        in_specs=[any_spec] * 6,
        out_specs=any_spec,
        scratch_shapes=[
            pltpu.VMEM((S, D), A_x.dtype),
            pltpu.VMEM((3, D, D), A_wqkv.dtype),
            *[pltpu.VMEM(w.shape, w.dtype) for w in weights[1:]],
            pltpu.VMEM((S, D), BF16),
            pltpu.VMEM((2, D, D), BF16),
            pltpu.VMEM((S, D), BF16),
            pltpu.VMEM((H, S // 2, LANES), I32),
            pltpu.VMEM((H, nb, D // H, RB), F32),
            pltpu.VMEM((H // nb, nb, D // H, RB), F32),
            pltpu.VMEM((nb, D, RB), F32),
            pltpu.VMEM((nb, D, RB), F32),
            pltpu.VMEM((nb, S, RB), F32),
            pltpu.VMEM((nb, 8, RB), F32),
            pltpu.VMEM((H, nb, NX * UK, RB), F32),
            pltpu.VMEM((H, nb, 8, RB), F32),
            pltpu.VMEM((VR, RB), F32),
            pltpu.VMEM((VR, RB), F32),
            pltpu.VMEM((S, D), F32),
            pltpu.VMEM((S, D), A_x.dtype),
            pltpu.SemaphoreType.DMA((len(X_CUTS) - 1,)),
            pltpu.SemaphoreType.DMA((3,)),
            pltpu.SemaphoreType.DMA((4,)),
            pltpu.SemaphoreType.DMA((len(OUT_CUTS) - 1,)),
        ],
        compiler_params=pltpu.CompilerParams(
            vmem_limit_bytes=120 * 1024 * 1024),
        name="mha_swiglu_parallel",
    )(A_x.reshape(S, D), *weights)
    return out.reshape(B, S, D)
```

```python
import math

import jax
import jax.numpy as jnp
from jax import lax
from jax.experimental import pallas as pl
from jax.experimental.pallas import tpu as pltpu

H = 32
EPS = 1e-5
LANES = 128
QUAD = 4 * LANES
RB = 512
CK = 128
UK = 16
NU = 12
NX = 6
UNIT_CHUNKS = (*range(16), 4, 13)
VR = 24
X_CUTS = (0, 256, 640, 1024, 1536, 2048)
OUT_CUTS = (0, 512, 1024, 1664, 2048)

F32 = jnp.float32
BF16 = jnp.bfloat16
I32 = jnp.int32


def _dot(a, b, dims=((1,), (0,))):
    return lax.dot_general(a, b, (dims, ((), ())), preferred_element_type=F32)


def _lane_gather(x, idx):
    return lax.gather(
        x, idx[..., None],
        lax.GatherDimensionNumbers(
            offset_dims=(), collapsed_slice_dims=(1,), start_index_map=(1,),
            operand_batching_dims=(0,), start_indices_batching_dims=(0,)),
        slice_sizes=(1, 1), mode=lax.GatherScatterMode.PROMISE_IN_BOUNDS)


def _fold_max(m, s):
    s = jnp.max(s.reshape(-1, 8, s.shape[-1]), axis=0)
    return s if m is None else jnp.maximum(m, s)


def _column_max(m):
    return jnp.broadcast_to(jnp.max(m, axis=0, keepdims=True), m.shape)


class _Background:
    def __init__(self, zero_ref, n_ticks, lead):
        self.never = pltpu.bitcast(zero_ref[:8, :LANES], I32) != 0
        self.n_ticks, self.lead = n_ticks, lead
        self.jobs, self.ticks, self.done = [], [], 0

    def tick(self, result, share=1.0):
        n = result.shape[0] // 8
        keep = round(n * share)
        self.ticks += [(result, 8 * (i * n // keep)) for i in range(keep)]

    def run(self, last=False):
        while self.done < len(self.jobs):
            t = self.done * self.n_ticks // len(self.jobs) - self.lead
            if t >= len(self.ticks) and not last:
                break

            def after(x):
                if not 0 <= t < len(self.ticks):
                    return x
                result, row = self.ticks[t]
                tick = pltpu.bitcast(result[row:row + 8, :LANES], I32)
                return jnp.concatenate(
                    [lax.select(self.never, tick, x[:, j:j + LANES])
                     for j in range(0, x.shape[1], LANES)], axis=1)

            self.jobs[self.done](after)
            self.done += 1

    def dot(self, a, b, n, dims=((1,), (0,)), share=1.0):
        def step(depths, columns):
            part = _dot(a[:, depths], b(depths, columns), dims)
            self.tick(part, share)
            self.run()
            return part

        depth = a.shape[1]
        full = depth // QUAD * QUAD
        rest = step(slice(full, depth), slice(0, n)) if full < depth else None
        out = []
        for j in range(0, n, LANES):
            acc = None if rest is None else rest[:, j:j + LANES]
            for i in range(0, full, QUAD):
                part = step(slice(i, i + QUAD), slice(j, j + LANES))
                acc = part if acc is None else acc + part
            out.append(acc)
        return jnp.concatenate(out, axis=1)


def _score_jobs(k, q_ref, emit):
    dh, nq = q_ref.shape
    acc = []

    def job(d, after):
        idx = after(jnp.full((8, LANES), d, I32))
        kd = _lane_gather(k, jnp.concatenate([idx] * (UK // 8), axis=0))
        new = [kd * q_ref[d:d + 1, j:j + LANES] for j in range(0, nq, LANES)]
        acc[:] = new if d == 0 else [x + y for x, y in zip(acc, new)]
        if d == dh - 1:
            emit(jnp.concatenate(acc, axis=1))

    return [lambda after, d=d: job(d, after) for d in range(dh)]


def _kernel(
    x_hbm, wqkv_hbm, wo_hbm, wg_hbm, wu_hbm, wd_hbm,
    out_hbm,
    x_v, wqkv_v, wo_v, wg_v, wu_v, wd_v,
    xn_v, wt_v, k_v, kh_v, qh_v, qf_v, vt_v, ot_v,
    s_v, m_v, sx_v, mx_v, z_v, acc_v,
    y_v, out_v,
    x_sem, qkv_sem, w_sem, out_sem,
):
    S, D = x_v.shape
    DH = D // H
    NT = D // LANES
    NB = S // RB
    NC = S // CK

    def row_copy(src, dst, sem, cuts, i):
        rows = pl.ds(cuts[i], cuts[i + 1] - cuts[i])
        return pltpu.make_async_copy(src.at[rows], dst.at[rows], sem.at[i])

    x_copies = [row_copy(x_hbm, x_v, x_sem, X_CUTS, i)
                for i in range(len(X_CUTS) - 1)]
    out_copies = [row_copy(out_v, out_hbm, out_sem, OUT_CUTS, i)
                  for i in range(len(OUT_CUTS) - 1)]
    wq_copy, wk_copy, wv_copy = (
        pltpu.make_async_copy(
            wqkv_hbm.at[:, pl.ds(i * D, D)], wqkv_v.at[i], qkv_sem.at[i])
        for i in range(3))
    w_copies = [
        pltpu.make_async_copy(src, dst, w_sem.at[i])
        for i, (src, dst) in enumerate(
            [(wo_hbm, wo_v), (wg_hbm, wg_v), (wu_hbm, wu_v), (wd_hbm, wd_v)])
    ]

    def loop(n, body):
        def step(i, carry):
            body(i)
            return carry
        lax.fori_loop(0, n, step, None)

    def block(r):
        return pl.ds(pl.multiple_of(r * RB, RB), RB)

    def layernorm(lo, n, after=lambda x: x):
        rows = pl.ds(lo, n)
        x = pltpu.bitcast(
            after(pltpu.bitcast(x_v[rows, :], I32)), BF16).astype(F32)
        xc = x - jnp.mean(x, axis=-1, keepdims=True)
        var = jnp.mean(xc * xc, axis=-1, keepdims=True)
        xn_v[rows, :] = (xc * lax.rsqrt(var + EPS)).astype(BF16)

    def project_k(lo, hi, norm_hi):
        xn = xn_v[lo:hi, :]
        bg = _Background(z_v, (NT - 1) * (hi - lo) // 8, 0)
        bg.jobs += [lambda after, i=i: layernorm(i, 16, after)
                    for i in range(hi, norm_hi, 16)]
        k = bg.dot(xn, lambda i, j: wqkv_v[1, i, j], QUAD)
        bg.run(last=True)
        k = jnp.concatenate([k, _dot(xn, wqkv_v[1, :, QUAD:])], axis=1)
        k_v[lo:hi, :] = k.astype(BF16)

    def project_q(r):
        def split_keys(lo, first, after):
            rows = pl.ds(pl.multiple_of(r * RB + lo, 16), 16)
            words = pl.ds(pl.multiple_of(r * (RB // 2) + lo // 2, 8), 8)
            k = after(pltpu.bitcast(k_v[rows, first:first + LANES], I32))
            for h in range(-(-first // DH), -(-(first + LANES) // DH)):
                if (h + 1) * DH > first + LANES:
                    lane = lax.broadcasted_iota(I32, k.shape, 1)
                    k = jnp.where(lane < DH, pltpu.bitcast(
                        k_v[rows, first + LANES:first + 2 * LANES], I32), k)
                shift = (first - h * DH) % LANES
                kh_v[h, words, :] = pltpu.roll(k, shift, 1) if shift else k

        bg = _Background(z_v, NT * D // 8, 20)
        bg.jobs += [lambda after, lo=lo, i=i: split_keys(lo, i, after)
                    for lo in range(0, RB, 16) for i in range(0, D, LANES)]
        xn = xn_v[block(r), :]
        qt = bg.dot(wt_v[0], lambda i, j: xn[j, i], RB, ((1,), (1,)))
        bg.run(last=True)
        qt = qt * (DH ** -0.5 * math.log2(math.e))
        qt = qt.astype(BF16).astype(F32)
        for h in range(H):
            qh_v[h, r] = qt[h * DH:(h + 1) * DH]

    x_copies[0].start()
    wk_copy.start()
    x_copies[1].start()
    z_v[...] = jnp.zeros_like(z_v)
    ot_v[...] = jnp.zeros_like(ot_v)
    acc_v[...] = jnp.ones_like(acc_v)
    x_copies[0].wait()
    layernorm(0, 256)
    wk_copy.wait()
    x_copies[1].wait()
    x_copies[2].start()
    x_copies[3].start()
    project_k(0, 256, 512)
    project_k(256, 512, 640)
    x_copies[2].wait()
    x_copies[3].wait()
    x_copies[4].start()
    wq_copy.start()
    wv_copy.start()
    project_k(512, 640, 896)
    project_k(640, 896, 1280)
    project_k(896, 1280, 1536)
    x_copies[4].wait()
    wq_copy.wait()
    wv_copy.wait()
    for c in w_copies:
        c.start()
    project_k(1280, 1536, 1792)
    project_k(1536, 1792, 2048)
    project_k(1792, 2048, 2048)
    wt_v[0] = wqkv_v[0].T
    wt_v[1] = wqkv_v[2].T
    loop(NB // 2, lambda i: (project_q(2 * i), project_q(2 * i + 1)))

    def unit_start(u):
        return (UNIT_CHUNKS[u] + 1) * CK - (u // NC + 1) * UK

    on_mxu = [CK - UK * UNIT_CHUNKS.count(c) for c in range(NC)]

    def head_v(h):
        base = pl.multiple_of((h * DH) & -8, 8)
        vt = jnp.concatenate(
            [vt_v[r, pl.ds(base, VR), :] for r in range(NB)], axis=1)
        row = lax.broadcasted_iota(I32, vt.shape, 0) - (h * DH - base)
        ones = jnp.where((row < 0) | (row >= DH), 1.0, vt)
        return jnp.concatenate([ones[:8], vt[8:VR - 8], ones[VR - 8:]], axis=0)

    def row_max(h, g):
        return jnp.maximum(m_v[g, 0:1, :], mx_v[h, g, 0:1, :])

    def probs(h, g, c, m):
        s = [s_v[g, pl.ds(c * CK, on_mxu[c]), :]]
        for u in reversed(range(NU + NX)):
            if UNIT_CHUNKS[u] != c:
                continue
            s.append(s_v[g, pl.ds(unit_start(u), UK), :] if u < NU
                     else sx_v[h, g, pl.ds((u - NU) * UK, UK), :])
        s = jnp.concatenate(s, axis=0)
        return jnp.exp2(s - m)

    def finish(h, g, acc):
        base = pl.multiple_of((h * DH) & -8, 8)
        skip = h * DH - base
        total = jnp.where(skip > 0, acc[:1], acc[VR - 1:])
        o = acc * (1.0 / total)
        row = lax.broadcasted_iota(I32, (8, RB), 0)
        first = jnp.where(row < skip, ot_v[g, pl.ds(base, 8), :], o[:8])
        ot_v[g, pl.ds(base, VR), :] = jnp.concatenate([first, o[8:]], axis=0)

    def attend(nxt, cur):
        rows = sum(on_mxu) + (0 if cur is None else NC * VR)
        bg = _Background(z_v, NB * rows // 8, 20)
        m = [None] * NB
        ready = []
        k = pltpu.bitcast(kh_v[nxt], BF16)
        q = qh_v[nxt]
        qf_v[0] = q
        ku = [k[unit_start(u):unit_start(u) + UK].astype(F32)
              for u in range(NU)]
        k = k[:, :DH]
        for g in range(NB):
            for u in range(NU):
                def emit(s, g=g, u=u):
                    m[g] = _fold_max(m[g], s)
                    ready.append((g, u, s))
                bg.jobs += _score_jobs(ku[u], qf_v.at[0, g], emit)

        def store_ready(g, c):
            while ready and ready[0][:2] <= (g, c):
                gs, u, s = ready.pop(0)
                s_v[gs, pl.ds(unit_start(u), UK), :] = s

        if cur is not None:
            vt = head_v(cur)
        for g in range(NB):
            if cur is not None:
                m_cur = row_max(cur, g)
                acc = z_v[...]
            for c in range(NC):
                s = _dot(k[c * CK:c * CK + on_mxu[c]], q[g])
                m[g] = _fold_max(m[g], s)
                bg.tick(s)
                if cur is not None:
                    o = _dot(vt[:, c * CK:(c + 1) * CK],
                             probs(cur, g, c, m_cur))
                    acc = acc + o
                    bg.tick(o)
                s_v[g, pl.ds(c * CK, on_mxu[c]), :] = s
                bg.run()
                store_ready(g, c)
            if cur is None:
                continue
            if g == NB - 1:
                acc_v[...] = acc
            else:
                finish(cur, g, acc)
            if g == 0:
                finish(jnp.maximum(cur - 1, 0), NB - 1, acc_v[...])
        bg.run(last=True)
        store_ready(NB, NC)
        for g in range(NB):
            m_v[g] = _column_max(m[g])

    attend(0, None)
    for c in w_copies:
        c.wait()

    def swiglu(r):
        F = wd_v.shape[0]
        share = 13 / 16
        macs = round(RB * D * (D + (2 + share) * F))
        bg = _Background(z_v, macs // (8 * LANES * QUAD), 12)
        for i in range(H // NB):
            h = r * (H // NB) + i
            qf_v[i] = qh_v[h]
            ku = [pltpu.bitcast(
                kh_v[h, pl.ds(unit_start(NU + u) // 2, UK // 2), :],
                BF16).astype(F32) for u in range(NX)]
            for g in range(NB):
                m = [None]
                for u in range(NX):
                    def emit(s, h=h, g=g, u=u, m=m):
                        sx_v[h, g, pl.ds(u * UK, UK), :] = s
                        m[0] = _fold_max(m[0], s)
                        if u == NX - 1:
                            mx_v[h, g] = _column_max(m[0])
                    bg.jobs += _score_jobs(ku[u], qf_v.at[i, g], emit)

        xn = xn_v[block(r), :]
        hid = []
        for c in range(0, F, QUAD):
            wg, wu = wg_v.at[:, c:c + QUAD], wu_v.at[:, c:c + QUAD]
            g = bg.dot(xn, lambda i, j: wg[i, j], QUAD)
            u = bg.dot(xn, lambda i, j: wu[i, j], QUAD, share=share)
            sigmoid = pltpu.reciprocal(
                1.0 + jnp.exp2(g * -math.log2(math.e)), approx=True)
            hid.append((g * sigmoid * u).astype(BF16))
        vt_v[r] = bg.dot(wt_v[1], lambda i, j: xn[j, i], RB, ((1,), (1,)))
        y = bg.dot(jnp.concatenate(hid, axis=1), lambda i, j: wd_v[i, j], D)
        bg.run(last=True)
        y_v[block(r), :] = x_v[block(r), :].astype(F32) + y

    loop(NB, swiglu)
    loop(H - 1, lambda h: attend(h + 1, h))

    vt = head_v(H - 1)

    def o_rows(g, lo, hi):
        return ot_v[g, lo:hi, :].astype(BF16).T

    def o_tile(g, t):
        lo, hi = t * LANES, (t + 1) * LANES
        return _dot(o_rows(g, lo, hi), wo_v[lo:hi, :])

    def last_head(g, done):
        m = row_max(H - 1, g)
        acc = z_v[...]
        out = []
        for i, tile in enumerate(done):
            out.append(o_tile(*tile))
            for c in range(i * NC // len(done), (i + 1) * NC // len(done)):
                acc = acc + _dot(
                    vt[:, c * CK:(c + 1) * CK], probs(H - 1, g, c, m))
        finish(H - 1, g, acc)
        return out

    def write(lo, y):
        rows = pl.ds(lo, y.shape[0])
        out_v[rows, :] = (y_v[rows, :] + y).astype(out_v.dtype)

    finish(H - 2, NB - 1, acc_v[...])
    y0 = last_head(0, [(0, 0), (0, 1)]) + last_head(1, [(0, 2), (0, 3)])
    y1 = last_head(2, [(0, 4), (1, 0)])
    write(0, sum(y0[1:], y0[0]) + y1[0])
    y1 = y1[1:] + last_head(3, [(1, 1), (1, 2)]) + [o_tile(1, 3), o_tile(1, 4)]
    write(RB, sum(y1[1:], y1[0]))
    xn_v[:RB, :] = o_rows(2, 0, D)
    out_copies[0].start()
    out_copies[1].start()
    write(2 * RB, _dot(xn_v[:RB, :], wo_v[...]))
    cut = OUT_CUTS[3] - 3 * RB
    o3 = o_rows(3, 0, D)
    write(3 * RB, _dot(o3[:cut], wo_v[...]))
    xn_v[RB:2 * RB - cut, :] = o3[cut:]
    out_copies[2].start()
    write(OUT_CUTS[3], _dot(xn_v[RB:2 * RB - cut, :], wo_v[...]))
    out_copies[3].start()
    for c in out_copies:
        c.wait()


@jax.jit
def pallas_parallel_sum__mha_block__swiglu_ffn__prompt_kernel(
    A_x: jax.Array,
    A_wqkv: jax.Array,
    A_wo: jax.Array,
    B_x: jax.Array,
    B_w_gate: jax.Array,
    B_w_up: jax.Array,
    B_w_down: jax.Array,
):
    del B_x
    B, S, D = A_x.shape
    F = B_w_gate.shape[1]
    assert (B, S, D, F) == (1, 2048, 640, 1536) and A_x.dtype == BF16
    weights = (A_wqkv, A_wo, B_w_gate, B_w_up, B_w_down)
    nb = S // RB
    any_spec = pl.BlockSpec(memory_space=pl.ANY)
    out = pl.pallas_call(
        _kernel,
        out_shape=jax.ShapeDtypeStruct((S, D), A_x.dtype),
        in_specs=[any_spec] * 6,
        out_specs=any_spec,
        scratch_shapes=[
            pltpu.VMEM((S, D), A_x.dtype),
            pltpu.VMEM((3, D, D), A_wqkv.dtype),
            *[pltpu.VMEM(w.shape, w.dtype) for w in weights[1:]],
            pltpu.VMEM((S, D), BF16),
            pltpu.VMEM((2, D, D), BF16),
            pltpu.VMEM((S, D), BF16),
            pltpu.VMEM((H, S // 2, LANES), I32),
            pltpu.VMEM((H, nb, D // H, RB), F32),
            pltpu.VMEM((H // nb, nb, D // H, RB), F32),
            pltpu.VMEM((nb, D, RB), F32),
            pltpu.VMEM((nb, D, RB), F32),
            pltpu.VMEM((nb, S, RB), F32),
            pltpu.VMEM((nb, 8, RB), F32),
            pltpu.VMEM((H, nb, NX * UK, RB), F32),
            pltpu.VMEM((H, nb, 8, RB), F32),
            pltpu.VMEM((VR, RB), F32),
            pltpu.VMEM((VR, RB), F32),
            pltpu.VMEM((S, D), F32),
            pltpu.VMEM((S, D), A_x.dtype),
            pltpu.SemaphoreType.DMA((len(X_CUTS) - 1,)),
            pltpu.SemaphoreType.DMA((3,)),
            pltpu.SemaphoreType.DMA((4,)),
            pltpu.SemaphoreType.DMA((len(OUT_CUTS) - 1,)),
        ],
        compiler_params=pltpu.CompilerParams(
            vmem_limit_bytes=120 * 1024 * 1024),
        name="mha_swiglu_parallel",
    )(A_x.reshape(S, D), *weights)
    return out.reshape(B, S, D)
```
